```python
import os as _os
_os.environ.setdefault('JAX_PLATFORMS', 'cpu')
import jax
import jax.numpy as jnp

def _softmax(x, axis=-1):
    return jax.nn.softmax(x, axis=axis)

def _gelu(x):
    return jax.nn.gelu(x, approximate=True)

def _silu(x):
    return jax.nn.silu(x)

def _sigmoid(x):
    return jax.nn.sigmoid(x)

def _layernorm(x, axis=-1, eps=1e-05):
    m = jnp.mean(x, axis=axis, keepdims=True)
    v = jnp.var(x, axis=axis, keepdims=True)
    return (x - m) / jnp.sqrt(v + eps)

def _scatter_add(tgt, idx, src, axis=0):
    return tgt.at[idx].add(src)

def _segment_sum(src, seg, n):
    return jax.ops.segment_sum(src, seg, n)

class _Rng:

    def __init__(self, key):
        self._k = key

    def _next(self):
        self._k, sub = jax.random.split(self._k)
        return sub

    def normal(self, shape):
        return jax.random.normal(self._next(), shape, dtype=jnp.bfloat16)

    def randint(self, lo, hi, shape):
        return jax.random.randint(self._next(), shape, lo, hi, dtype=jnp.int32)

    def uniform(self, shape, lo=0.0, hi=1.0):
        return jax.random.uniform(self._next(), shape, jnp.bfloat16, lo, hi)

    def permutation(self, n):
        return jax.random.permutation(self._next(), n)
kernel_name = 'gated_mix__sliding_block__memory_aug_recurrent_mem_tr__prompt'

def setup_inputs():
    _rng = _Rng(jax.random.key(int.from_bytes(__import__("os").urandom(4), "little")))
    _w = lambda a: (lambda t: t.astype(jnp.bfloat16) if jnp.issubdtype(t.dtype, jnp.floating) else t)(jnp.asarray(a))

    def _A_setup():
        B, S, D = (1, 2048, 448)
        return {'x': _w((lambda *s: _rng.normal(s) * 0.05)(B, S, D)), 'wqkv': _w((lambda *s: _rng.normal(s) * 0.8)(D, 3 * D)), 'wo': _w((lambda *s: _rng.normal(s) * 0.05)(D, D))}
    _A_in = _A_setup()

    def _B_setup():
        B, S, Dm = (1, 2048, 448)
        H, Dh = (16, 256)
        M, seg = (8, 32)
        seg = min(seg, S)
        S = S // seg * seg
        return {'x': _w((lambda *s: _rng.normal(s) * 0.05)(B, S, Dm)), 'mem0': _w((lambda *s: _rng.normal(s) * 0.8)(B, M, Dm)), 'Wq': _w((lambda *s: _rng.normal(s) * 3.2)(Dm, H, Dh) * Dm ** (-0.5)), 'Wk': _w((lambda *s: _rng.normal(s) * 3.2)(Dm, H, Dh) * Dm ** (-0.5)), 'Wv': _w((lambda *s: _rng.normal(s) * 0.8)(Dm, H, Dh) * Dm ** (-0.5)), 'Wo': _w((lambda *s: _rng.normal(s) * 0.8)(H, Dh, Dm) * (H * Dh) ** (-0.5)), 'seg_len': seg}
    _B_in = _B_setup()
    return {'A_x': _A_in['x'], 'A_wqkv': _A_in['wqkv'], 'A_wo': _A_in['wo'], 'B_x': _B_in['x'], 'B_mem0': _B_in['mem0'], 'B_Wq': _B_in['Wq'], 'B_Wk': _B_in['Wk'], 'B_Wv': _B_in['Wv'], 'B_Wo': _B_in['Wo'], 'B_seg_len': _B_in['seg_len'], 'gate_w': _w((lambda *s: _rng.normal(s) * 0.05)(448) * 16.0)}

def reference(A_x, A_wqkv, A_wo, B_x, B_mem0, B_Wq, B_Wk, B_Wv, B_Wo, B_seg_len, gate_w):

    def _A_ref(x, wqkv, wo):
        B, S, D = x.shape
        H = 16
        Dh = D // H
        W = 256
        qkv = (lambda x, *d: x.transpose(*d))((x @ wqkv).reshape(B, S, 3, H, Dh), 2, 0, 3, 1, 4)
        q, k, v = (qkv[0], qkv[1], qkv[2])
        scores = jnp.einsum('bhqd,bhkd->bhqk', q, k) * Dh ** (-0.5)
        idx = jnp.arange(S)
        mask = (idx[:, None] - idx[None, :] >= 0) & (idx[:, None] - idx[None, :] < W)
        scores = jnp.where(mask[None, None], scores, -1000000000.0)
        p = _softmax(scores, axis=-1)
        o = jnp.einsum('bhqk,bhkd->bhqd', p, v)
        return (lambda x, *d: x.transpose(*d))(o, 0, 2, 1, 3).reshape(B, S, D) @ wo

    def _B_ref(x, mem0, Wq, Wk, Wv, Wo, seg_len):
        B, S, Dm = x.shape
        H, Dh = (Wq.shape[1], Wq.shape[2])
        M = mem0.shape[1]
        scale = Dh ** (-0.5)
        n_seg = S // seg_len
        L = M + seg_len
        idx = jnp.arange(L)
        mask = (idx[:, None] < M) | (idx[:, None] >= idx[None, :])
        mem = mem0
        outs = []
        for s in range(n_seg):
            xs = x[:, s * seg_len:(s + 1) * seg_len, :].copy()
            h = jnp.concatenate([mem, xs], axis=1)
            q = jnp.einsum('btd,dhe->bhte', h, Wq)
            k = jnp.einsum('btd,dhe->bhte', h, Wk)
            v = jnp.einsum('btd,dhe->bhte', h, Wv)
            scores = jnp.einsum('bhqe,bhke->bhqk', q, k) * scale
            scores = jnp.where(mask[None, None], scores, -1000000000.0)
            p = _softmax(scores, axis=-1)
            o = jnp.einsum('bhqk,bhke->bhqe', p, v)
            o = jnp.einsum('bhte,hed->btd', o, Wo)
            mem = o[:, :M, :].copy()
            outs.append(o[:, M:, :])
        return jnp.concatenate(outs, axis=1)
    x = A_x
    g = _sigmoid((x * gate_w).sum(-1, keepdims=True))
    a = _A_ref(x, A_wqkv, A_wo)
    b = _B_ref(x, B_mem0, B_Wq, B_Wk, B_Wv, B_Wo, B_seg_len)
    return g * a + (1 - g) * b
```

```python
import jax
import jax.numpy as jnp
from jax import lax
import jax.experimental.pallas as pl
import jax.experimental.pallas.tpu as pltpu

S = 2048
D = 448
DP = 512
NEG = -1e30
LOG2E = 1.4426950408889634
bf16 = jnp.bfloat16
f32 = jnp.float32
u32 = jnp.uint32

NQB = S // 128
NSEG = 64
SEG = 32
MEM = 8
E = 256
H = 16
CH = 896
BULK_UNROLL = 4


def _iota(shape, dim):
    return lax.broadcasted_iota(jnp.int32, shape, dim)


def _dot(a, b):
    return jnp.dot(a, b, preferred_element_type=f32)


def _dot_nt(a, b):
    return lax.dot_general(a, b, (((1,), (1,)), ((), ())), preferred_element_type=f32)


def _kernel(xat_hbm, wqkv_hbm, wo_hbm, mem_hbm, wq_hbm, wk_hbm, wv_hbm, wot_hbm, gw_hbm,
            out_hbm,
            wqkv_s, wo_s, xat_s, gw_s, mem_s,
            wq0, wq1, wk0, wk1, wv0, wv1, wot_s,
            wt_s, wopt_s, qt_s, k_s, vt_s, gt_s, s_s, at_s, bb_s, ost_s,
            x_s, xq_s, wcat_s, ybulk_s, ystep_s, m_s,
            in_sems, out_sems):
    def cp(src, dst, i):
        return pltpu.make_async_copy(src, dst, in_sems.at[i])

    c_wqkv = cp(wqkv_hbm, wqkv_s, 0)
    c_wo = cp(wo_hbm, wo_s, 1)
    c_gw = cp(gw_hbm, gw_s, 2)

    def c_xat(j):
        c0 = j * 512 if isinstance(j, int) else pl.multiple_of(j * 512, 512)
        return pltpu.make_async_copy(xat_hbm.at[:, pl.ds(c0, 512)], xat_s.at[0:D, pl.ds(c0, 512)], in_sems.at[13 + j])

    c_mem = cp(mem_hbm, mem_s, 5)
    c_w = []
    for i, (src, dsts) in enumerate(((wq_hbm, (wq0, wq1)), (wk_hbm, (wk0, wk1)), (wv_hbm, (wv0, wv1)))):
        for j in range(2):
            c_w.append(cp(src.at[:, pl.ds(128 * j, 128)], dsts[j], 6 + 2 * i + j))
    c_wot = cp(wot_hbm, wot_s, 12)
    for c in (c_wqkv, c_xat(0), c_wo, c_gw, c_xat(1), c_xat(2), c_xat(3), c_mem):
        c.start()

    r = _iota((128, 128), 0)
    c = _iota((128, 128), 1)
    lane128 = _iota((256, 128), 1)
    kpad = pltpu.bitcast(jnp.where((lane128 & 31) == 28, NEG, 0.0).astype(bf16), u32)
    for h in range(H):
        k_s[h, 0:128, :] = kpad
    vt_s[0] = jnp.zeros((4, 128, 128), bf16)
    vt_s[1] = jnp.zeros((4, 128, 128), bf16)
    xat_s[D:DP, :] = jnp.zeros((DP - D, S), bf16)
    at_s[...] = jnp.zeros(at_s.shape, f32)
    bb_s[...] = jnp.zeros(bb_s.shape, f32)

    c_wqkv.wait()

    def src_tile(st):
        lo = 128 * st
        hi = min(lo + 128, 3 * D)
        w = wqkv_s[:, lo:hi]
        if hi - lo < 128:
            w = jnp.concatenate([w, jnp.zeros((D, 128 - (hi - lo)), bf16)], axis=1)
        return w

    def sel(t, st):
        cp_ = 128 * t + r
        src = 28 * (cp_ >> 5) + (cp_ & 31)
        return jnp.where((src == 128 * st + c) & ((cp_ & 31) < 28), 1.0, 0.0).astype(bf16)

    def hit(t, st):
        return [cc for cc in range(4)
                if 112 * t + 28 * cc < 128 * st + 128 and 112 * t + 28 * cc + 28 > 128 * st]

    for t in range(12):
        acc = [None] * 4
        for st in range((112 * t) // 128, (112 * t + 111) // 128 + 1):
            cs = hit(t, st)
            p = _dot_nt(sel(t, st)[32 * cs[0]:32 * cs[-1] + 32], src_tile(st))
            for k, cc in enumerate(cs):
                pk = p[32 * k:32 * k + 32]
                acc[cc] = pk if acc[cc] is None else acc[cc] + pk
        wt_s[128 * t:128 * t + 128, 0:D] = jnp.concatenate(acc, axis=0).astype(bf16)
    c_gw.wait()
    wt_s[1536:1552, 0:D] = jnp.broadcast_to(gw_s[...].reshape(1, D), (16, D))
    wt_s[:, D:DP] = jnp.zeros((1552, DP - D), bf16)
    c_wo.wait()
    for t in range(4):
        acc = None
        for st in range((112 * t) // 128, (112 * t + 111) // 128 + 1):
            lo = 128 * st
            hi = min(lo + 128, D)
            w = wo_s[lo:hi, :]
            if hi - lo < 128:
                w = jnp.concatenate([w, jnp.zeros((128 - (hi - lo), D), bf16)], axis=0)
            p = _dot(sel(t, st), w)
            acc = p if acc is None else acc + p
        accp = jnp.concatenate([acc, jnp.zeros((128, DP - D), f32)], axis=1)
        wopt_s[t] = accp.T.astype(bf16)

    for cw in c_w:
        cw.start()
    c_wot.start()

    cA = (28.0 ** -0.5) * LOG2E

    def proj(i, carry):
        c0 = pl.multiple_of(i * 128, 128)
        xb = xat_s[:, pl.ds(c0, 128)]
        x_s[pl.ds(c0, 128), :] = xb.T
        row = _iota((DP, 128), 0)
        is28 = (row & 31) == 28
        kt = _dot(wt_s[512:1024, :], xb)
        for t in range(4):
            ktt = pltpu.bitcast(kt[128 * t:128 * t + 128].T.astype(bf16), u32)
            rolled = [ktt] + [pltpu.roll(ktt, 32 * k, 1) for k in range(1, 4)]
            for cc in range(4):
                for g in range(4):
                    w0 = pl.multiple_of(i * 64 + 128 - 16 * g, 16)
                    k_s[4 * t + cc, pl.ds(w0, 64), 32 * g:32 * g + 32] = rolled[(g - cc) % 4][:, 32 * g:32 * g + 32]
        gl = _dot(wt_s[1536:1552, :], xb)
        gt_s[i] = jax.nn.sigmoid(gl[0:8])
        qt = _dot(wt_s[0:512, :], xb)
        qt = jnp.where(is28, 1.0, qt * cA)
        lg = _iota((32, 128), 1) >> 5
        for h in range(H):
            q = qt[32 * h:32 * h + 32]
            q4 = jnp.concatenate([jnp.where(lg == g, q, 0.0) for g in range(4)], axis=0)
            qt_s[i, h] = pltpu.bitcast(q4.astype(bf16), u32)
        vt = _dot(wt_s[1024:1536, :], xb)
        vt_s[i + 2] = jnp.where(is28, 1.0, vt).astype(bf16).reshape(4, 128, 128)
        return carry

    def proj4(j, carry):
        c_xat(j).wait()
        for q in range(4):
            proj(4 * j + q, carry)
        return carry
    lax.fori_loop(0, 4, proj4, 0)

    cB = (256.0 ** -0.5) * LOG2E
    z64 = jnp.zeros((64, E), bf16)

    def put(j, lo, w):
        n = w.shape[1]
        wb = pltpu.bitcast(w.astype(bf16), u32)
        wcat_s[j, 0:224, lo:lo + n] = wb
        wcat_s[j, 224:256, lo:lo + n] = wb[192:224]

    def heads(halves, a2, b):
        off = pl.multiple_of(4 * a2, 4)
        ev, od = [], []
        for hv in halves:
            wu = hv.bitcast(u32).at[pl.ds(off, 3580), :]
            words = wu[pl.ds(b, D, stride=8), :]
            ev.append(pltpu.bitcast(words << 16, f32))
            od.append(pltpu.bitcast(words & jnp.uint32(0xFFFF0000), f32))
        return jnp.concatenate(ev, axis=1), jnp.concatenate(od, axis=1)

    def nt_parts(l_e, l_o, r_e, r_o):
        x_e = _dot_nt(l_e, r_e[0:384].astype(bf16))
        zl = jnp.zeros((64, E), bf16)
        m_e = _dot_nt(r_e[384:448].astype(bf16), jnp.concatenate([l_e, zl], axis=0))
        m_o = _dot_nt(r_o[384:448].astype(bf16), jnp.concatenate([l_o, zl], axis=0))
        x_o = _dot_nt(l_o, r_o[0:384].astype(bf16))
        x_m = jnp.concatenate([m_e, m_o], axis=0).T[0:D]
        return x_e, x_m, x_o

    def pre_t(a2, carry):
        for b in range(4):
            p = 4 * a2 + b
            wq_e, wq_o = heads((wq0, wq1), a2, b)
            wk_e, wk_o = heads((wk0, wk1), a2, b)
            a_e, a_m, a_o = nt_parts(wq_e.astype(bf16), wq_o.astype(bf16), wk_e, wk_o)
            put(p, 0, a_e * cB)
            put(p, 384, a_m * cB)
            put(p, 512, a_o * cB)
        return carry

    def pre_u(a2, carry):
        for k in range(2):
            w0 = heads((wv0, wv1), a2, 2 * k)
            w1 = heads((wv0, wv1), a2, 2 * k + 1)
            for par in range(2):
                h0 = 8 * a2 + 4 * k + par
                b_e, b_m, b_o = nt_parts(w0[par].astype(bf16), w1[par].astype(bf16), wot_s[h0], wot_s[h0 + 2])
                j = 8 + 4 * a2 + 2 * k + par
                put(j, 0, b_e)
                put(j, 384, b_m)
                put(j, 512, b_o)
        return carry

    for cw in c_w[0:4]:
        cw.wait()
    lax.fori_loop(0, 2, pre_t, 0)
    for cw in c_w[4:6]:
        cw.wait()
    c_wot.wait()
    lax.fori_loop(0, 2, pre_u, 0)

    for q in range(4):
        xq_s[128 * q:128 * q + 128, :] = jnp.concatenate(
            [x_s[32 * (16 * q + s) + 24:32 * (16 * q + s) + 32, :] for s in range(16)], axis=0)

    def bulk(j, carry):
        w = pltpu.bitcast(wcat_s[j], bf16)
        for q in range(4):
            ybulk_s[j, 128 * q:128 * q + 128, :] = _dot(xq_s[128 * q:128 * q + 128, :], w)
        return carry
    lax.fori_loop(0, 16, bulk, 0, unroll=BULK_UNROLL)

    c_mem.wait()
    m_s[:, 0:D] = mem_s[...].astype(f32)
    m_s[:, D:DP] = jnp.zeros((MEM, DP - D), f32)
    z8 = jnp.zeros((8, 128), f32)

    def out_copy(slot, grp):
        c0 = pl.multiple_of(grp * 128, 128)
        return pltpu.make_async_copy(ost_s.at[slot, 0:D, :], out_hbm.at[:, pl.ds(c0, 128)], out_sems.at[grp])

    def mix(par, t, grp, slot):
        r0 = t * 128 if isinstance(t, int) else pl.multiple_of(t * 128, 128)
        bt = bb_s[par, t].T
        at = at_s[par, pl.ds(r0, 128), :]
        g = gt_s[grp, 0:1, :]
        ost_s[slot, pl.ds(r0, 128), :] = (bt + g * (at - bt)).astype(bf16)

    def a_scores(u, piece):
        qb = u >> 2
        t = u & 3
        w0 = pl.multiple_of(qb * 64 + 48 * piece, 16)
        for cc in range(4):
            kt = pltpu.bitcast(k_s[4 * t + cc, pl.ds(w0, 48), :], bf16)
            q4 = pltpu.bitcast(qt_s[qb, 4 * t + cc], bf16)
            s_s[96 * piece:96 * piece + 96, 128 * cc:128 * cc + 128] = _dot(kt, q4)

    def a_soft(cc):
        kb_i = _iota((32, 128), 0)
        qa_i = _iota((32, 128), 1) & 31
        tri = kb_i > qa_i
        lo = 128 * cc
        sc = jnp.where(tri, s_s[0:32, lo:lo + 128], s_s[256:288, lo:lo + 128])
        s1 = s_s[32:256, lo:lo + 128]
        mx = jnp.maximum(jnp.max(sc, axis=0, keepdims=True), jnp.max(s1, axis=0, keepdims=True))
        pc = jnp.exp2(sc - mx)
        p1 = jnp.exp2(s1 - mx)
        blks = ([jnp.where(tri, pc, 0.0)] + [p1[32 * j:32 * j + 32] for j in range(7)]
                + [jnp.where(tri, 0.0, pc)])
        lg = _iota((32, 128), 1) >> 5
        zero = jnp.zeros((32, 128), f32)
        blk = lambda j: blks[j] if 0 <= j < 9 else zero
        y = {j: jnp.where(lg >= 2, blk(j - 2), blk(j)) for j in range(0, 11)}
        yk = lambda j: y[j] if 0 <= j < 11 else zero
        z = [jnp.where((lg & 1) == 1, yk(j - 1), yk(j)) for j in range(12)]
        return [jnp.concatenate(z[4 * kb:4 * kb + 4], axis=0).astype(bf16) for kb in range(3)]

    def a_pv(qb, t, cc, ps):
        ot = (_dot(vt_s[qb, t, 32 * cc:32 * cc + 32, :], ps[0])
              + _dot(vt_s[qb + 1, t, 32 * cc:32 * cc + 32, :], ps[1])
              + _dot(vt_s[qb + 2, t, 32 * cc:32 * cc + 32, :], ps[2]))
        inv = 1.0 / ot[28:29, :]
        return ot * inv

    for piece in range(3):
        a_scores(0, piece)

    def step(qb, t):
        s = 4 * qb + t
        par = qb & 1
        r0 = pl.multiple_of(s * SEG, SEG)
        b0 = pl.multiple_of(s * 8, 8)
        m2 = m_s[...]
        xs = x_s[pl.ds(r0, SEG), :].astype(f32)
        lhs = jnp.concatenate([xs[0:24], m2], axis=0).astype(bf16)
        mr = m2[:, 384:512]
        mr = jnp.where(_iota((MEM, 128), 1) < 64, mr + pltpu.roll(mr, 64, 1), 0.0)
        m = jnp.concatenate([m2[:, 0:384], mr], axis=1)

        def chunk(j):
            ystep_s[j] = _dot(lhs, pltpu.bitcast(wcat_s[j], bf16))

        h40 = jnp.concatenate([xs, m], axis=0)
        h48b = jnp.concatenate([h40[:, 0:384], jnp.zeros((8, 384), f32)], axis=0).astype(bf16)
        hrem = h40[:, 384:512]
        hrem2 = jnp.concatenate([hrem, pltpu.roll(hrem, 64, 1)], axis=0).astype(bf16)

        def xg(j, lo, n):
            return [ystep_s[j, 0:8, lo:lo + n], ystep_s[j, 8:16, lo:lo + n], ystep_s[j, 16:24, lo:lo + n],
                    ybulk_s[j, pl.ds(b0, 8), lo:lo + n]]

        def mg(j, lo, n):
            return ystep_s[j, 24:32, lo:lo + n]

        def cat(gs):
            return jnp.concatenate(gs, axis=0)

        def tchunk(gam, c):
            return 4 * gam + c

        def uchunk(gam, c, par):
            return 8 + 4 * gam + 2 * (c >> 1) + par

        kj = _iota((40, 128), 0)
        ln = _iota((40, 128), 1)
        mask = (kj >= 32) | (kj <= (ln & 31))
        st = [None] * 5
        pt = [None] * 5

        def b_scores(gam):
            tm = cat([r_ for c in range(4) for r_ in xg(tchunk(gam, c), 384, 128)])
            r2 = _dot(hrem2, tm.T.astype(bf16))
            for par in range(2):
                tt = cat([r_ for c in range(4) for r_ in xg(tchunk(gam, c), 512 * par, 384)])
                st[2 * gam + par] = _dot(h48b, tt.T.astype(bf16))[0:40] + r2[40 * par:40 * par + 40]

        def b_scores_m():
            order = [(c, g >> 1, g & 1) for c in range(4) for g in range(4)]
            tm = cat([mg(tchunk(gam, c), 384, 128) for c, gam, par in order])
            r2 = _dot(hrem2, tm.T.astype(bf16))
            rr = jnp.where(((ln >> 3) & 1) == 0, r2[0:40], r2[40:80])
            tt = cat([mg(tchunk(gam, c), 512 * par, 384) for c, gam, par in order])
            st[4] = _dot(h48b, tt.T.astype(bf16))[0:40] + rr

        def b_soft(g):
            x = jnp.where(mask, st[g], NEG) if g < 4 else st[g]
            mx = jnp.max(x, axis=0, keepdims=True)
            p = jnp.exp2(x - mx)
            l = jnp.sum(p, axis=0, keepdims=True)
            pt[g] = p * (1.0 / l)

        lhs_k = {}

        def b_trans():
            l32 = _iota((32, 128), 1)
            l8 = _iota((8, 128), 1)
            m1 = cat([pt[g][0:32] for g in range(4)]).T
            m2_ = cat([jnp.where((l8 >> 5) == c, pt[g][32:40], 0.0) for c in range(4) for g in range(4)]).T
            m3 = cat([jnp.where(((l32 >> 3) & 3) == g, pt[4][0:32], 0.0) for g in range(4)]).T
            m4 = cat([jnp.where((l8 >> 3) == q, pt[4][32:40], 0.0) for q in range(16)]).T
            for c in range(4):
                mq = (m3[32 * c:32 * c + 8] + m3[32 * c + 8:32 * c + 16]) + (m3[32 * c + 16:32 * c + 24] + m3[32 * c + 24:32 * c + 32])
                lhs_k[c] = cat([m1[32 * c:32 * c + 32], mq])
            xq = (m2_[0:32] + m2_[32:64]) + (m2_[64:96] + m2_[96:128])
            parts = [m4[8 * q:8 * q + 8] for q in range(16)]
            while len(parts) > 1:
                parts = [parts[i] + parts[i + 1] for i in range(0, len(parts), 2)]
            lhs_k[4] = cat([xq, parts[0]])

        acc = {}

        def add(key, v):
            acc[key] = v if key not in acc else acc[key] + v

        def b_pv(k):
            gs = [(g >> 1, g & 1) for g in range(4)]
            lhs_m = jnp.concatenate([cat([lhs_k[c], z8]) for c in (2 * k, 2 * k + 1)], axis=1).astype(bf16)
            u_m = cat([r_ for c in (2 * k, 2 * k + 1) for gam, par in gs
                       for r_ in xg(uchunk(gam, c, par), 512 * (c & 1), 384)]).astype(bf16)
            add('m', _dot(lhs_m, u_m))
            lhs_r = cat([lhs_k[2 * k], lhs_k[2 * k + 1]]).astype(bf16)
            u_r = cat([r_ for gam, par in gs for r_ in xg(uchunk(gam, 2 * k, par), 384, 128)]).astype(bf16)
            add('r', _dot(lhs_r, u_r))

        def b_pv_m():
            order = [(c, g >> 1, g & 1) for c in range(4) for g in range(4)]
            u_m = cat([mg(uchunk(gam, c, par), 512 * (c & 1), 384) for c, gam, par in order]).astype(bf16)
            add('m', _dot(cat([lhs_k[4], z8]).astype(bf16), u_m))
            l40 = _iota((40, 128), 1)
            even = ((l40 >> 5) & 1) == 0
            lhs_r = cat([jnp.where(even, lhs_k[4], 0.0), jnp.where(even, 0.0, lhs_k[4])]).astype(bf16)
            u_r = cat([mg(uchunk(gam, c, par), 384, 128) for c, gam, par in order]).astype(bf16)
            add('r', _dot(lhs_r, u_r))

        ots = []
        aps = {}
        un = jnp.minimum(s + 1, NSEG - 1)
        aps[0] = a_soft(0)
        chunk(0)
        aps[1] = a_soft(1)
        chunk(1)
        ots.append(a_pv(qb, t, 0, aps[0]))
        aps[2] = a_soft(2)
        chunk(2)
        ots.append(a_pv(qb, t, 1, aps[1]))
        aps[3] = a_soft(3)
        chunk(3)
        ots.append(a_pv(qb, t, 2, aps[2]))
        chunk(4)
        ots.append(a_pv(qb, t, 3, aps[3]))
        chunk(5)
        b_scores(0)
        chunk(6)
        b_soft(0)
        b_soft(1)
        chunk(7)
        ot = jnp.concatenate(ots, axis=0).astype(bf16)
        ao = _dot(wopt_s[t, 0:D, :], ot)
        at_s[par, 0:D, :] = ao if t == 0 else at_s[par, 0:D, :] + ao
        chunk(8)
        chunk(9)
        b_scores(1)
        mix(1 - par, t, jnp.maximum(qb - 1, 0), qb)
        chunk(12)
        b_scores_m()
        b_soft(2)
        b_soft(3)
        chunk(13)
        b_soft(4)
        b_trans()
        chunk(10)
        chunk(11)
        chunk(14)
        b_pv(0)
        chunk(15)
        a_scores(un, 0)
        a_scores(un, 1)
        b_pv(1)
        b_pv_m()
        a_scores(un, 2)
        o_main = acc['m']
        o_rem2 = acc['r']
        m_s[:, 0:384] = o_main[32:40]
        m_s[:, 384:512] = jnp.where(_iota((MEM, 128), 1) < 64, o_rem2[32:40], o_rem2[72:80])
        o_rem = o_rem2[0:32] + pltpu.roll(o_rem2[40:72], 64, 1)
        t32 = t * 32
        for n in range(3):
            bb_s[par, n, t32:t32 + 32, :] = o_main[0:32, 128 * n:128 * n + 128]
        bb_s[par, 3, t32:t32 + 32, :] = o_rem

    def group(qb, carry):
        for t in range(4):
            step(qb, t)

        @pl.when(qb >= 1)
        def _():
            out_copy(qb, qb - 1).start()
        return carry
    lax.fori_loop(0, NQB, group, 0)

    for t in range(4):
        mix((NQB - 1) & 1, t, NQB - 1, NQB)
    out_copy(NQB, NQB - 1).start()
    for g in range(NQB):
        out_copy(g + 1, g).wait()


@jax.jit
def _run(A_x, A_wqkv, A_wo, B_mem0, B_Wq, B_Wk, B_Wv, B_Wo, gate_w):
    xat = jnp.swapaxes(A_x, 1, 2)[0]
    wot = jnp.swapaxes(B_Wo, 1, 2)
    wq = B_Wq.reshape(D * H, E)
    wk = B_Wk.reshape(D * H, E)
    wv = B_Wv.reshape(D * H, E)
    any_spec = pl.BlockSpec(memory_space=pl.ANY)
    half = pltpu.VMEM((D * H, 128), bf16)
    scratch = [
        pltpu.VMEM((D, 3 * D), bf16), pltpu.VMEM((D, D), bf16), pltpu.VMEM((DP, S), bf16),
        pltpu.VMEM((D,), bf16), pltpu.VMEM((MEM, D), bf16),
        half, half, half, half, half, half, pltpu.VMEM((H, D, E), bf16),
        pltpu.VMEM((1552, DP), bf16), pltpu.VMEM((4, DP, 128), bf16),
        pltpu.VMEM((NQB, H, 64, 128), u32), pltpu.VMEM((H, (S + 256) // 2, 128), u32),
        pltpu.VMEM((NQB + 2, 4, 128, 128), bf16), pltpu.VMEM((NQB, 8, 128), f32),
        pltpu.VMEM((288, 512), f32), pltpu.VMEM((2, DP, 128), f32),
        pltpu.VMEM((2, 4, 128, 128), f32), pltpu.VMEM((NQB + 1, DP, 128), bf16),
        pltpu.VMEM((S, DP), bf16), pltpu.VMEM((512, DP), bf16), pltpu.VMEM((16, 256, CH), u32),
        pltpu.VMEM((16, 512, CH), f32), pltpu.VMEM((16, 32, CH), f32), pltpu.VMEM((MEM, DP), f32),
        pltpu.SemaphoreType.DMA((17,)), pltpu.SemaphoreType.DMA((NQB,)),
    ]
    out_t = pl.pallas_call(
        _kernel,
        out_shape=jax.ShapeDtypeStruct((D, S), bf16),
        in_specs=[any_spec] * 9,
        out_specs=any_spec,
        scratch_shapes=scratch,
        compiler_params=pltpu.CompilerParams(vmem_limit_bytes=120 * 1024 * 1024),
    )(xat, A_wqkv, A_wo, B_mem0[0], wq, wk, wv, wot, gate_w)
    return jnp.swapaxes(out_t[None], 1, 2)


def pallas_gated_mix__sliding_block__memory_aug_recurrent_mem_tr__prompt_kernel(
    A_x, A_wqkv, A_wo, B_x, B_mem0, B_Wq, B_Wk, B_Wv, B_Wo, B_seg_len, gate_w,
):
    del B_x
    if isinstance(B_seg_len, int):
        assert B_seg_len == SEG
    assert A_x.shape == (1, S, D)
    return _run(A_x, A_wqkv, A_wo, B_mem0, B_Wq, B_Wk, B_Wv, B_Wo, gate_w)
```
